```python
import os as _os
_os.environ.setdefault('JAX_PLATFORMS', 'cpu')
import jax
import jax.numpy as jnp

def _softmax(x, axis=-1):
    return jax.nn.softmax(x, axis=axis)

def _gelu(x):
    return jax.nn.gelu(x, approximate=True)

def _silu(x):
    return jax.nn.silu(x)

def _sigmoid(x):
    return jax.nn.sigmoid(x)

def _layernorm(x, axis=-1, eps=1e-05):
    m = jnp.mean(x, axis=axis, keepdims=True)
    v = jnp.var(x, axis=axis, keepdims=True)
    return (x - m) / jnp.sqrt(v + eps)

def _scatter_add(tgt, idx, src, axis=0):
    return tgt.at[idx].add(src)

def _segment_sum(src, seg, n):
    return jax.ops.segment_sum(src, seg, n)

class _Rng:

    def __init__(self, key):
        self._k = key

    def _next(self):
        self._k, sub = jax.random.split(self._k)
        return sub

    def normal(self, shape):
        return jax.random.normal(self._next(), shape, dtype=jnp.bfloat16)

    def randint(self, lo, hi, shape):
        return jax.random.randint(self._next(), shape, lo, hi, dtype=jnp.int32)

    def uniform(self, shape, lo=0.0, hi=1.0):
        return jax.random.uniform(self._next(), shape, jnp.bfloat16, lo, hi)

    def permutation(self, n):
        return jax.random.permutation(self._next(), n)
kernel_name = 'standalone__conformer_conv_module__speech'

def setup_inputs():
    _rng = _Rng(jax.random.key(int.from_bytes(__import__("os").urandom(4), "little")))
    _w = lambda a: (lambda t: t.astype(jnp.bfloat16) if jnp.issubdtype(t.dtype, jnp.floating) else t)(jnp.asarray(a))
    B, T, D, K = (2, 16000, 256, 5)
    return {'x': _w((lambda *s: _rng.normal(s) * 0.2)(B, T, D)), 'w_pw1': _w((lambda *s: _rng.normal(s) * 0.2)(D, 2 * D)), 'dw': _w((lambda *s: _rng.normal(s) * 0.05)(K, D)), 'w_pw2': _w((lambda *s: _rng.normal(s) * 0.05)(D, D))}

def reference(x, w_pw1, dw, w_pw2):
    B, T, D = x.shape
    K = dw.shape[0]
    h = x @ w_pw1
    a, b = (h[..., :D].copy(), h[..., D:].copy())
    h = a * _sigmoid(b)
    pad = K // 2
    hp = jnp.pad(h, ((0, 0), (pad, pad), (0, 0)))
    out = jnp.zeros_like(h)
    for i in range(K):
        out = out + hp[:, i:i + T, :] * dw[i][None, None, :]
    return _silu(out) @ w_pw2
```

```python
import functools
import jax, jax.numpy as jnp
import jax.experimental.pallas as pl
import jax.experimental.pallas.tpu as pltpu

def build(C=400, S=80, LOOK=2, A=16, order="il", nobc=True):
    def f(x, w_pw1, dw, w_pw2):
        B, T, D = x.shape
        K = dw.shape[0]
        assert D == 256 and K == 5
        H = D // 2
        nT = T // C
        NB = B * nT
        assert NB % 2 == 0 and T % C == 0 and C % S == 0 and S % 16 == 0
        R = B * T
        CK = A + 8
        nS = C // S
        bf, f32, u32 = jnp.bfloat16, jnp.float32, jnp.uint32
        def kernel(x_hbm, w1_hbm, dw_hbm, w2_hbm, o_hbm,
                   xlo, xhi, ob, alo, ahi, blo, bhi, w1b, w2b, dwb, dws, xsem, osem, wsem):
            def xcopies(j):
                r = pl.multiple_of(j * C, 16)
                return (pltpu.make_async_copy(x_hbm.at[pl.ds(r, C), pl.ds(0, H)], xlo.at[pl.ds(r, C), :], xsem.at[j]),
                        pltpu.make_async_copy(x_hbm.at[pl.ds(r, C), pl.ds(H, H)], xhi.at[pl.ds(r, C), :], xsem.at[j]))
            def ocopy(j):
                r = pl.multiple_of(j * C, 16)
                return pltpu.make_async_copy(ob.at[pl.ds(r, C), :], o_hbm.at[pl.ds(r, C), :], osem)
            wc = [pltpu.make_async_copy(w1_hbm.at[:, pl.ds(n * H, H)], w1b.at[n], wsem) for n in range(4)]
            wc += [pltpu.make_async_copy(w2_hbm.at[:, pl.ds(n * H, H)], w2b.at[n], wsem) for n in range(2)]
            wc += [pltpu.make_async_copy(dw_hbm, dwb, wsem)]
            for c in wc: c.start()
            for j in range(0, min(LOOK + 1, NB)):
                for c in xcopies(j): c.start()
            for c in wc: c.wait()
            for n in (2, 3):
                w1b[n] = (w1b[n].astype(f32) * 0.5).astype(bf)
            dwf = dwb[...].astype(f32) * 0.25
            for k in range(K):
                dws[2 * k] = jnp.broadcast_to(dwf[k:k+1, 0:H], (8, H))
                dws[2 * k + 1] = jnp.broadcast_to(dwf[k:k+1, H:], (8, H))
            def ld(ref, *idx):
                return pltpu.bitcast(ref.bitcast(u32)[idx], bf)
            def wtile(ref, n):
                return ld(ref, n, slice(None), slice(None))
            def glu(r2, n):
                xv = jnp.concatenate([ld(xlo, pl.ds(r2, n // 2), slice(None)), ld(xhi, pl.ds(r2, n // 2), slice(None))], axis=1)
                out = []
                for m in (0, 1):
                    w = jnp.concatenate([wtile(w1b, m), wtile(w1b, m + 2)], axis=1)
                    h = jnp.dot(xv, w, preferred_element_type=f32)
                    out.append(h[:, :H] * (jnp.tanh(h[:, H:]) + 1.0))
                return out
            def conv(g, half, p):
                o = None
                for k in range(K):
                    t = g[p - 2 + k : p - 2 + k + S, :].reshape(S // 8, 8, H) * dws[2 * k + half]
                    o = t if o is None else o + t
                o = o.reshape(S, H)
                return o * (jnp.tanh(o) + 1.0)
            def p2(j, s, rb):
                r = pl.multiple_of(j * C + s * S, 16)
                p = CK - A + s * S
                sv = jnp.concatenate([conv(rb[0], 0, p), conv(rb[1], 1, p)], axis=1).astype(bf)
                w = jnp.concatenate([wtile(w2b, 0), wtile(w2b, 1)], axis=1)
                ob[pl.ds(r, S), :] = jnp.dot(sv, w, preferred_element_type=f32).astype(bf)
            def p1(j, s, wb, carry):
                r2 = pl.multiple_of((j * C + A + s * S) // 2, 8) if A % 16 == 0 else (j * C + A + s * S) // 2
                g = glu(r2, S)
                if s == 0:
                    first = (j % nT) == 0
                    for m in (0, 1):
                        c = carry[m]
                        wb[m][0:8, :] = jnp.where(first, 0.0, c[0:8])
                        wb[m][8:CK, :] = c[8:CK]
                if s == nS - 1:
                    last = ((j + 1) % nT) == 0
                    carry = [g[m][S - CK:, :] for m in (0, 1)]
                    for m in (0, 1):
                        wb[m][CK + s * S : CK + s * S + S - A, :] = g[m][:S - A]
                        wb[m][CK + C - A : CK + C, :] = jnp.where(last, 0.0, g[m][S - A:])
                else:
                    for m in (0, 1):
                        wb[m][CK + s * S : CK + (s + 1) * S, :] = g[m]
                return carry
            def half(j, wb, rb, carry, do_p1=True, do_p2=True, static=False):
                if do_p1:
                    if static:
                        if j + 1 + LOOK < NB:
                            for c in xcopies(j + 1 + LOOK): c.start()
                        if j + 1 < NB:
                            for c in xcopies(j + 1): c.wait()
                    else:
                        @pl.when(j + 1 + LOOK < NB)
                        def _():
                            for c in xcopies(j + 1 + LOOK): c.start()
                        for c in xcopies(j + 1): c.wait()
                if order == "il":
                    for s in range(nS):
                        if do_p1: carry = p1(j, s, wb, carry)
                        if do_p2: p2(j - 1, s, rb)
                elif order == "il2":
                    for s in range(nS):
                        if do_p2: p2(j - 1, s, rb)
                        if do_p1: carry = p1(j, s, wb, carry)
                elif order == "convfirst":
                    if do_p2:
                        for s in range(nS): p2(j - 1, s, rb)
                    if do_p1:
                        for s in range(nS): carry = p1(j, s, wb, carry)
                elif order == "seq":
                    if do_p1:
                        for s in range(nS): carry = p1(j, s, wb, carry)
                    if do_p2:
                        for s in range(nS): p2(j - 1, s, rb)
                if do_p2: ocopy(j - 1).start()
                return carry
            Ab, Bb = (alo, ahi), (blo, bhi)
            for c in xcopies(0): c.wait()
            g0 = glu(0, 16)
            z = jnp.zeros((8, H), f32)
            carry = [jnp.concatenate([z, g0[m][:A]], axis=0) for m in (0, 1)]
            carry = half(0, Ab, None, carry, do_p2=False, static=True)
            def body(i, carry):
                j = 2 * i + 1
                carry = half(j, Bb, Ab, carry)
                carry = half(j + 1, Ab, Bb, carry)
                return carry
            carry = jax.lax.fori_loop(0, NB // 2 - 1, body, carry)
            carry = half(NB - 1, Bb, Ab, carry, static=True)
            half(NB, None, Bb, carry, do_p1=False, static=True)
            def wbody(j, _):
                ocopy(j).wait()
            jax.lax.fori_loop(0, NB, wbody, None)
        out = pl.pallas_call(
            kernel,
            in_specs=[pl.BlockSpec(memory_space=pl.ANY)] * 4,
            out_specs=pl.BlockSpec(memory_space=pl.ANY),
            out_shape=jax.ShapeDtypeStruct((R, D), bf),
            scratch_shapes=[pltpu.VMEM((R + 16, H), bf), pltpu.VMEM((R + 16, H), bf), pltpu.VMEM((R, D), bf)]
                         + [pltpu.VMEM((C + CK + 8, H), f32)] * 4 + [
                            pltpu.VMEM((4, D, H), bf), pltpu.VMEM((2, D, H), bf),
                            pltpu.VMEM((K, D), bf), pltpu.VMEM((2 * K, 8, H), f32),
                            pltpu.SemaphoreType.DMA((NB,)), pltpu.SemaphoreType.DMA(()), pltpu.SemaphoreType.DMA(())],
            compiler_params=pltpu.CompilerParams(vmem_limit_bytes=100 * 1024 * 1024, disable_bounds_checks=nobc),
        )(x.reshape(R, D), w_pw1, dw, w_pw2)
        return out.reshape(B, T, D)
    return f


_IMPL = build(C=800, S=160, order="seq")


@jax.jit
def pallas_standalone__conformer_conv_module__speech_kernel(x, w_pw1, dw, w_pw2):
    return _IMPL(x, w_pw1, dw, w_pw2)
```

```python
import jax
import jax.numpy as jnp
import jax.experimental.pallas as pl
import jax.experimental.pallas.tpu as pltpu

_C = 320
_HALO = 8
_PRO = 20
_PRO_WAITS = (1, 3, 7)
_U = 40
_LAST_SPLIT = 4


def _conformer_kernel(x_hbm, w1_hbm, dw_hbm, w2_hbm, o_hbm,
                      xb, ob, alo, ahi, blo, bhi, w1b, w2b, dwb, dws,
                      xsem, wsem, osem, order_sem, *, T, K):
    R, D = xb.shape
    H = D // 2
    C, U, P = _C, _U, _PRO
    nT = T // C
    NB = R // C
    n_it = (NB - P) // U
    f32, bf16 = jnp.float32, jnp.bfloat16
    bufs = ((alo, ahi), (blo, bhi))
    zeros = jnp.zeros((_HALO, H), f32)

    cuts = (0,) + _PRO_WAITS + (P,)
    n_pro = len(cuts) - 1

    def x_copy(row0, rows, sem_idx):
        return pltpu.make_async_copy(
            x_hbm.at[pl.ds(row0, rows), :], xb.at[pl.ds(row0, rows), :], xsem.at[sem_idx])

    def pro_copy(i):
        return x_copy(cuts[i] * C, (cuts[i + 1] - cuts[i]) * C, i)

    def loop_copy(i):
        row0 = (P + U * i) * C
        if not isinstance(row0, int):
            row0 = pl.multiple_of(row0, 16)
        return x_copy(row0, U * C, n_pro + i)

    def out_copy(row0, rows):
        return pltpu.make_async_copy(
            ob.at[pl.ds(row0, rows), :], o_hbm.at[pl.ds(row0, rows), :], osem)

    w1_copy = pltpu.make_async_copy(w1_hbm, w1b, wsem.at[0])
    w2_copies = (pltpu.make_async_copy(w2_hbm, w2b, wsem.at[1]),
                 pltpu.make_async_copy(dw_hbm, dwb, wsem.at[2]))

    def in_order():
        pl.semaphore_signal(order_sem, 1)
        pl.semaphore_wait(order_sem, 1)

    pro_copy(0).start()
    w1_copy.start()
    in_order()
    pro_copy(1).start()
    for c in w2_copies:
        c.start()
    for i in range(2, n_pro):
        in_order()
        pro_copy(i).start()
    in_order()
    loop_copy(0).start()

    alo[0:_HALO, :] = zeros
    ahi[0:_HALO, :] = zeros

    def pick(pred, v):
        if isinstance(pred, bool):
            return zeros if pred else v
        return jnp.where(pred, 0.0, v)

    def glu(h, cur, other):
        row0 = h * C
        if not isinstance(row0, int):
            row0 = pl.multiple_of(row0, 16)
        xv = xb[pl.ds(row0, C), :]
        head = []
        for m in range(2):
            w = jnp.concatenate([w1b[:, m * H:(m + 1) * H],
                                 w1b[:, D + m * H:D + (m + 1) * H]], axis=1)
            hh = jnp.dot(xv, w, preferred_element_type=f32)
            g = hh[:, :H] * (jnp.tanh(hh[:, H:] * 0.5) + 1.0)
            cur[m][_HALO:_HALO + C, :] = g
            if not (isinstance(h, int) and h == 0):
                other[m][_HALO + C:, :] = pick(h % nT == 0, g[:_HALO])
            head.append(pick((h + 1) % nT == 0, g[C - _HALO:]))
        return head

    def conv_silu(g, m):
        o = None
        for k in range(K):
            p = _HALO - K // 2 + k
            t = g[p:p + C, :].reshape(C // 8, 8, H) * dws[2 * k + m]
            o = t if o is None else o + t
        o = o.reshape(C, H)
        return o * (jnp.tanh(o) + 1.0)

    def conv_pw2(j, src, send, pieces=1):
        row0 = j * C
        if not isinstance(row0, int):
            row0 = pl.multiple_of(row0, 16)
        s = jnp.concatenate([conv_silu(src[m], m) for m in range(2)], axis=1).astype(bf16)
        y = jnp.dot(s, w2b[...], preferred_element_type=f32).astype(ob.dtype)
        q = C // pieces
        for u in range(pieces):
            ob[pl.ds(row0 + u * q, q), :] = y[u * q:(u + 1) * q]
            if send:
                out_copy(row0 + u * q, q).start()

    def step(h, parity, send):
        cur, other = bufs[parity], bufs[1 - parity]
        head = glu(h, cur, other)
        if not (isinstance(h, int) and h == 0):
            conv_pw2(h - 1, other, send)
        for m in range(2):
            other[m][0:_HALO, :] = head[m]

    for h in range(P):
        if h in cuts:
            pro_copy(cuts.index(h)).wait()
        if h == 0:
            w1_copy.wait()
        if h == 1:
            for c in w2_copies:
                c.wait()
            dwf = dwb[...].astype(f32) * 0.25
            for k in range(K):
                for m in range(2):
                    dws[2 * k + m] = jnp.broadcast_to(dwf[k:k + 1, m * H:(m + 1) * H], (8, H))
        step(h, h % 2, send=False)
    out_copy(0, (P - 1) * C).start()

    def body(i, carry):
        @pl.when(i + 1 < n_it)
        def _():
            loop_copy(i + 1).start()

        loop_copy(i).wait()
        h0 = P + U * i
        for u in range(U):
            step(h0 + u, (P + u) % 2, send=True)
        return carry

    jax.lax.fori_loop(0, n_it, body, 0)

    last = bufs[(NB - 1) % 2]
    for m in range(2):
        last[m][_HALO + C:, :] = zeros
    conv_pw2(NB - 1, last, send=True, pieces=_LAST_SPLIT)

    pltpu.make_async_copy(ob, o_hbm, osem).wait()


@jax.jit
def pallas_standalone__conformer_conv_module__speech_kernel(
    x: jax.Array,
    w_pw1: jax.Array,
    dw: jax.Array,
    w_pw2: jax.Array,
):
    B, T, D = x.shape
    K = dw.shape[0]
    R = B * T
    H = D // 2
    assert D == 256 and K // 2 <= _HALO and K % 2 == 1
    assert T % _C == 0 and (R // _C - _PRO) % _U == 0 and R // _C > _PRO
    n_pieces = len(_PRO_WAITS) + 1 + (R // _C - _PRO) // _U

    def kernel_function(*refs):
        _conformer_kernel(*refs, T=T, K=K)

    glu_buf = pltpu.VMEM((_C + 2 * _HALO, H), jnp.float32)
    out = pl.pallas_call(
        kernel_function,
        in_specs=[pl.BlockSpec(memory_space=pl.ANY)] * 4,
        out_specs=pl.BlockSpec(memory_space=pl.ANY),
        out_shape=jax.ShapeDtypeStruct((R, D), x.dtype),
        scratch_shapes=[
            pltpu.VMEM((R, D), x.dtype),
            pltpu.VMEM((R, D), x.dtype),
            glu_buf, glu_buf, glu_buf, glu_buf,
            pltpu.VMEM((D, 2 * D), w_pw1.dtype),
            pltpu.VMEM((D, D), w_pw2.dtype),
            pltpu.VMEM((K, D), dw.dtype),
            pltpu.VMEM((2 * K, 8, H), jnp.float32),
            pltpu.SemaphoreType.DMA((n_pieces,)),
            pltpu.SemaphoreType.DMA((3,)),
            pltpu.SemaphoreType.DMA(()),
            pltpu.SemaphoreType.REGULAR,
        ],
        compiler_params=pltpu.CompilerParams(
            vmem_limit_bytes=64 * 1024 * 1024,
            disable_bounds_checks=True,
        ),
    )(x.reshape(R, D), w_pw1, dw, w_pw2)
    return out.reshape(B, T, D)
```
